```python
import os as _os
_os.environ.setdefault("JAX_PLATFORMS", "cpu")
import jax
import jax.numpy as jnp

def _softmax(x, axis=-1):
    return jax.nn.softmax(x, axis=axis)
def _gelu(x):
    return jax.nn.gelu(x, approximate=True)
def _silu(x):
    return jax.nn.silu(x)
def _sigmoid(x):
    return jax.nn.sigmoid(x)
def _layernorm(x, axis=-1, eps=1e-5):
    m = jnp.mean(x, axis=axis, keepdims=True)
    v = jnp.var(x, axis=axis, keepdims=True)
    return (x - m) / jnp.sqrt(v + eps)
def _scatter_add(tgt, idx, src, axis=0):
    return tgt.at[idx].add(src)
def _segment_sum(src, seg, n):
    return jax.ops.segment_sum(src, seg, n)
class _Rng:
    def __init__(self, key):
        self._k = key
    def _next(self):
        self._k, sub = jax.random.split(self._k)
        return sub
    def normal(self, shape):
        return jax.random.normal(self._next(), shape, dtype=jnp.bfloat16)
    def randint(self, lo, hi, shape):
        return jax.random.randint(self._next(), shape, lo, hi, dtype=jnp.int32)
    def uniform(self, shape, lo=0.0, hi=1.0):
        return jax.random.uniform(self._next(), shape, jnp.bfloat16, lo, hi)
    def permutation(self, n):
        return jax.random.permutation(self._next(), n)


kernel_name = 'standalone__instancenorm__sampling'

def setup_inputs():
    _rng = _Rng(jax.random.key(int.from_bytes(__import__("os").urandom(4), "little")))
    _w = (lambda a: (lambda t: t.astype(jnp.bfloat16) if jnp.issubdtype(t.dtype, jnp.floating) else t)(jnp.asarray(a)))
    B, C, H, W = 16, 640, 16, 32
    return {
        "x": _w((lambda *s: _rng.normal(s) * 0.05)(B, C, H, W)),
        "g": _w((lambda *s: _rng.normal(s) * 0.05)(C) + 1.0),
        "b": _w((lambda *s: _rng.normal(s) * 0.05)(C)),
    }

def reference(x, g, b):
    mu = x.mean(axis=(-2, -1), keepdims=True)
    var = ((x - mu) * (x - mu)).mean(axis=(-2, -1), keepdims=True)
    xhat = (x - mu) / jnp.sqrt(var + 1e-5)
    return xhat * g.reshape(1, -1, 1, 1) + b.reshape(1, -1, 1, 1)
```

```python
import jax
import jax.numpy as jnp
import jax.experimental.pallas as pl
import jax.experimental.pallas.tpu as pltpu

_EPS = 1e-5


def _make_kernel(B, HW, C, k_start):
    def kernel(x_hbm, g_hbm, b_hbm, o_hbm, buf, gv, bv, rsem, wsem, gsem):
        def rd(i):
            return pltpu.make_async_copy(
                x_hbm.at[pl.ds(i * HW, HW)], buf.at[i], rsem.at[i])

        def wr(i):
            return pltpu.make_async_copy(
                buf.at[i], o_hbm.at[pl.ds(i * HW, HW)], wsem.at[i])

        cg = pltpu.make_async_copy(g_hbm, gv, gsem.at[0])
        cb = pltpu.make_async_copy(b_hbm, bv, gsem.at[1])
        cg.start()
        cb.start()
        jax.lax.fori_loop(0, B, lambda i, _: rd(i).start(), None)
        cg.wait()
        cb.wait()
        g = gv[...].astype(jnp.float32).reshape(1, C)
        b = bv[...].astype(jnp.float32).reshape(1, C)

        def step(i):
            xf = buf[i].astype(jnp.float32)
            mu = jnp.sum(xf, axis=0, keepdims=True) * (1.0 / HW)
            d = xf - mu
            var = jnp.sum(d * d, axis=0, keepdims=True) * (1.0 / HW)
            s = jax.lax.rsqrt(var + _EPS) * g
            buf[i] = (d * s + b).astype(buf.dtype)

        def body1(i, _):
            rd(i).wait()
            step(i)

        jax.lax.fori_loop(0, k_start, body1, None)
        rd(k_start).wait()
        jax.lax.fori_loop(0, k_start, lambda j, _: wr(j).start(), None)
        step(k_start)
        wr(k_start).start()

        def body3(i, _):
            rd(i).wait()
            step(i)
            wr(i).start()

        jax.lax.fori_loop(k_start + 1, B, body3, None)
        jax.lax.fori_loop(0, B, lambda j, _: wr(j).wait(), None)

    return kernel


@jax.jit
def pallas_standalone__instancenorm__sampling_kernel(
    x: jax.Array,
    g: jax.Array,
    b: jax.Array,
):
    B, C, H, W = x.shape
    HW = H * W
    xt = jnp.transpose(x, (0, 2, 3, 1)).reshape(B * HW, C)
    anyspec = pl.BlockSpec(memory_space=pl.ANY)
    out = pl.pallas_call(
        _make_kernel(B, HW, C, B - 2),
        in_specs=[anyspec, anyspec, anyspec],
        out_specs=anyspec,
        out_shape=jax.ShapeDtypeStruct((B * HW, C), x.dtype),
        scratch_shapes=[
            pltpu.VMEM((B, HW, C), x.dtype),
            pltpu.VMEM((C,), g.dtype),
            pltpu.VMEM((C,), b.dtype),
            pltpu.SemaphoreType.DMA((B,)),
            pltpu.SemaphoreType.DMA((B,)),
            pltpu.SemaphoreType.DMA((2,)),
        ],
        compiler_params=pltpu.CompilerParams(vmem_limit_bytes=64 * 1024 * 1024),
    )(xt, g, b)
    return jnp.transpose(out.reshape(B, H, W, C), (0, 3, 1, 2))
```

```python
import jax
import jax.numpy as jnp
import jax.experimental.pallas as pl
import jax.experimental.pallas.tpu as pltpu

_EPS = 1e-5


def _make_kernel(B, HW, C):
    K = max(B - 2, 0)
    WSEM = K % 2
    inv_n = 1.0 / HW

    def kernel(x_hbm, g_hbm, b_hbm, o_hbm, buf, g_vmem, b_vmem, sem):
        def read(i):
            return pltpu.make_async_copy(
                x_hbm.at[pl.ds(i * HW, HW)], buf.at[pl.ds(i * HW, HW)], sem.at[i % 2]
            )

        def write(i, n=1):
            return pltpu.make_async_copy(
                buf.at[pl.ds(i * HW, n * HW)],
                o_hbm.at[pl.ds(i * HW, n * HW)],
                sem.at[WSEM],
            )

        copy_g = pltpu.make_async_copy(g_hbm, g_vmem, sem.at[0])
        copy_b = pltpu.make_async_copy(b_hbm, b_vmem, sem.at[0])
        copy_g.start()
        copy_b.start()
        jax.lax.fori_loop(0, min(2, B), lambda i, _: read(i).start(), None)
        copy_g.wait()
        copy_b.wait()
        read(0).wait()

        gamma = g_vmem[...].astype(jnp.float32).reshape(1, C)
        beta = b_vmem[...].astype(jnp.float32).reshape(1, C)

        def body(i, _):
            @pl.when(i > 0)
            def _():
                read(i).wait()

            @pl.when(i + 2 < B)
            def _():
                read(i + 2).start()

            if K > 0:

                @pl.when(i == K)
                def _():
                    write(0, K).start()

            rows = pl.ds(pl.multiple_of(i * HW, HW), HW)
            x = buf[rows, :].astype(jnp.float32)
            mu = jnp.sum(x, axis=0, keepdims=True) * inv_n
            d = x - mu
            var = jnp.sum(d * d, axis=0, keepdims=True) * inv_n
            scale = jax.lax.rsqrt(var + _EPS) * gamma
            buf[rows, :] = (d * scale + beta).astype(buf.dtype)

            @pl.when(i >= K)
            def _():
                write(i).start()

        jax.lax.fori_loop(0, B, body, None)
        write(0, B).wait()

    return kernel


@jax.jit
def pallas_standalone__instancenorm__sampling_kernel(
    x: jax.Array,
    g: jax.Array,
    b: jax.Array,
):
    B, C, H, W = x.shape
    HW = H * W
    x2d = jnp.transpose(x, (0, 2, 3, 1)).reshape(B * HW, C)
    any_spec = pl.BlockSpec(memory_space=pl.ANY)
    out = pl.pallas_call(
        _make_kernel(B, HW, C),
        in_specs=[any_spec, any_spec, any_spec],
        out_specs=any_spec,
        out_shape=jax.ShapeDtypeStruct((B * HW, C), x.dtype),
        scratch_shapes=[
            pltpu.VMEM((B * HW, C), x.dtype),
            pltpu.VMEM((C,), g.dtype),
            pltpu.VMEM((C,), b.dtype),
            pltpu.SemaphoreType.DMA((2,)),
        ],
        compiler_params=pltpu.CompilerParams(vmem_limit_bytes=64 * 1024 * 1024),
    )(x2d, g, b)
    return jnp.transpose(out.reshape(B, H, W, C), (0, 3, 1, 2))
```
